```python
import jax
import jax.numpy as jnp

def _softmax(x, axis=-1):
    return jax.nn.softmax(x, axis=axis)
def _gelu(x):
    return jax.nn.gelu(x, approximate=True)
def _silu(x):
    return jax.nn.silu(x)
def _sigmoid(x):
    return jax.nn.sigmoid(x)
def _layernorm(x, axis=-1, eps=1e-5):
    m = jnp.mean(x, axis=axis, keepdims=True)
    v = jnp.var(x, axis=axis, keepdims=True)
    return (x - m) / jnp.sqrt(v + eps)
def _scatter_add(tgt, idx, src, axis=0):
    return tgt.at[idx].add(src)
def _segment_sum(src, seg, n):
    return jax.ops.segment_sum(src, seg, n)
class _Rng:
    def __init__(self, key):
        self._k = key
    def _next(self):
        self._k, sub = jax.random.split(self._k)
        return sub
    def normal(self, shape):
        return jax.random.normal(self._next(), shape, dtype=jnp.bfloat16)
    def randint(self, lo, hi, shape):
        return jax.random.randint(self._next(), shape, lo, hi, dtype=jnp.int32)
    def uniform(self, shape, lo=0.0, hi=1.0):
        return jax.random.uniform(self._next(), shape, jnp.bfloat16, lo, hi)
    def permutation(self, n):
        return jax.random.permutation(self._next(), n)


kernel_name = 'interleave_layers__sliding_local_dilated__glu_gated_geglu__prompt'

def setup_inputs():
    _rng = _Rng(jax.random.key(int.from_bytes(__import__("os").urandom(4), "little")))
    _w = (lambda a: (lambda t: t.astype(jnp.bfloat16) if jnp.issubdtype(t.dtype, jnp.floating) else t)(jnp.asarray(a)))
    def _A_setup():
        B, S, D = 1, 2048, 576
        return {
            "x": _w((lambda *s: _rng.normal(s) * 0.05)(B, S, D)),
            "wqkv": _w((lambda *s: _rng.normal(s) * 0.05)(D, 3 * D)),
            "wo": _w((lambda *s: _rng.normal(s) * 0.05)(D, D)),
        }
    _A_in = _A_setup()

    def _B_setup():
        B, S, Dm, Df = 1, 2048, 576, 4608
        return {
            "x": _w((lambda *s: _rng.normal(s) * 0.05)(B, S, Dm)),
            "w_gate": _w((lambda *s: _rng.normal(s) * 0.05)(Dm, Df) * (Dm ** -0.5)),
            "w_up": _w((lambda *s: _rng.normal(s) * 0.05)(Dm, Df) * (Dm ** -0.5)),
            "w_down": _w((lambda *s: _rng.normal(s) * 0.05)(Df, Dm) * (Df ** -0.5)),
        }
    _B_in = _B_setup()

    return {
        "A_x": _A_in["x"],
        "A_wqkv": _A_in["wqkv"],
        "A_wo": _A_in["wo"],
        "B_x": _B_in["x"],
        "B_w_gate": _B_in["w_gate"],
        "B_w_up": _B_in["w_up"],
        "B_w_down": _B_in["w_down"],
    }

def reference(A_x, A_wqkv, A_wo, B_x, B_w_gate, B_w_up, B_w_down):
    def _A_ref(x, wqkv, wo):
        B, S, D = x.shape
        H = 32; Dh = D // H
        W, dil = 8, 2
        qkv = (lambda x, *d: x.transpose(*d))((x @ wqkv).reshape(B, S, 3, H, Dh), 2, 0, 3, 1, 4)
        q, k, v = qkv[0], qkv[1], qkv[2]
        scale = Dh ** -0.5
        pos = jnp.arange(S)
        off = jnp.arange(W) * dil
        idx = pos[:, None] - off[None, :]
        mask = idx >= 0
        idx_c = jnp.where(mask, idx, 0).reshape(-1)
        kg = k[:, :, idx_c, :].reshape(B, H, S, W, Dh)
        vg = v[:, :, idx_c, :].reshape(B, H, S, W, Dh)
        logits = jnp.einsum("bhsd,bhswd->bhsw", q, kg) * scale
        logits = jnp.where(mask[None, None, :, :], logits, -1e9)
        attn = _softmax(logits, axis=-1)
        o = jnp.einsum("bhsw,bhswd->bhsd", attn, vg)
        return (lambda x, *d: x.transpose(*d))(o, 0, 2, 1, 3).reshape(B, S, D) @ wo

    def _B_ref(x, w_gate, w_up, w_down):
        g = jnp.einsum("bsd,df->bsf", x, w_gate)
        u = jnp.einsum("bsd,df->bsf", x, w_up)
        h = _gelu(g) * u
        return jnp.einsum("bsf,fd->bsd", h, w_down)

    x = A_x
    x = x + _A_ref(_layernorm(x, axis=-1), A_wqkv, A_wo)
    x = x + _B_ref(_layernorm(x, axis=-1), B_w_gate, B_w_up, B_w_down)
    x = x + _A_ref(_layernorm(x, axis=-1), A_wqkv, A_wo)
    x = x + _B_ref(_layernorm(x, axis=-1), B_w_gate, B_w_up, B_w_down)
    return x
```

```python
import functools
import numpy as np
import jax
import jax.numpy as jnp
import jax.experimental.pallas as pl
import jax.experimental.pallas.tpu as pltpu

S, D, F = 2048, 576, 4608
H, DH, W = 32, 18, 8
EPS = 1e-5
SCALE = DH ** -0.5
C0 = 0.7978845608028654
HALO = 16
NT_DIMS = (((1,), (1,)), ((), ()))
f32, bf16 = jnp.float32, jnp.bfloat16


def _gelu(g):
    return 0.5 * g * (1.0 + jnp.tanh(C0 * (g + 0.044715 * (g * g * g))))


def _ln_t(x):
    m = jnp.mean(x, axis=0, keepdims=True)
    xc = x - m
    v = jnp.mean(xc * xc, axis=0, keepdims=True)
    return xc * jax.lax.rsqrt(v + EPS)


def build(T=512, FC=512, KA=3, R=64, order=None, staged=True):
    NB = S // T
    NC = F // FC

    def kernel(xT_hbm, wqkv_hbm, wo_hbm, wg_hbm, wu_hbm, wdT_hbm, outT_hbm,
               xin, xres, wqkv_raw, wo_raw, tmp, wpT, woT, wg, wu, wdT,
               qkv, obuf, xhat, outbuf, sems):
        def cp_x(b):
            return pltpu.make_async_copy(xT_hbm.at[:, pl.ds(b * T, T)], xin.at[:, pl.ds(b * T, T)], sems.at[b])
        cp_wqkv = pltpu.make_async_copy(wqkv_hbm, wqkv_raw, sems.at[NB])
        cp_wo = pltpu.make_async_copy(wo_hbm, wo_raw, sems.at[NB + 1])
        cp_wg = pltpu.make_async_copy(wg_hbm, wg, sems.at[NB + 2])
        cp_wu = pltpu.make_async_copy(wu_hbm, wu, sems.at[NB + 3])
        cp_wd = pltpu.make_async_copy(wdT_hbm, wdT, sems.at[NB + 4])
        def cp_out(r0):
            return pltpu.make_async_copy(outbuf.at[:, pl.ds(r0, T)], outT_hbm.at[:, pl.ds(r0, T)], sems.at[NB + 5])

        cp_wqkv.start()
        cp_x(0).start()
        if not staged:
            cp_wo.start()
            for b in range(1, NB):
                cp_x(b).start()
            cp_wg.start(); cp_wu.start(); cp_wd.start()

        qkv[:, pl.ds(0, HALO), :] = jnp.zeros((15, HALO, 128), f32)
        wpT[pl.ds(1728, 64), :] = jnp.zeros((64, D), bf16)
        woT[:, pl.ds(512, 128)] = jnp.zeros((D, 128), bf16)

        cp_wqkv.wait()
        if staged:
            cp_wo.start()
            for b in range(1, NB):
                cp_x(b).start()
            cp_wg.start(); cp_wu.start(); cp_wd.start()

        for c in range(5):
            n = 128 if c < 4 else 64
            tmp[c, :, pl.ds(0, n)] = wqkv_raw[pl.ds(c * 128, n), :].astype(f32).T
        for p in range(3):
            for d in range(DH):
                if d < 16:
                    row = p * 512 + d * 32
                else:
                    row = 1536 + p * 64 + (d - 16) * 32
                for c in range(5):
                    n = 128 if c < 4 else 64
                    rows = tmp[c, pl.ds(p * D + d, H, stride=DH), :]
                    wpT[pl.ds(row, H), pl.ds(c * 128, n)] = rows[:, :n].astype(bf16)

        def relayout_wo():
            cp_wo.wait()
            for c in range(5):
                n = 128 if c < 4 else 64
                tmp[c, pl.ds(0, D), pl.ds(0, n)] = wo_raw[:, pl.ds(c * 128, n)].astype(f32)
            for c in range(5):
                n = 128 if c < 4 else 64
                rows = jnp.concatenate(
                    [tmp[c, pl.ds(d, H, stride=DH), :] for d in range(DH)], axis=0)
                woT[pl.ds(c * 128, n), pl.ds(0, D)] = rows[:, :n].astype(bf16).T

        def load_x(b):
            cp_x(b).wait()
            xres[:, pl.ds(b * T, T)] = xin[:, pl.ds(b * T, T)].astype(f32)

        lane = jax.lax.broadcasted_iota(jnp.int32, (T, 128), 1)

        def stage_a(r0, first_wo=False):
            x = xres[:, pl.ds(r0, T)]
            xh = _ln_t(x).astype(bf16).T
            y = jax.lax.dot_general(xh, wpT[...], NT_DIMS, preferred_element_type=f32)
            rows = pl.ds(HALO + r0, T)
            for i in range(4):
                qkv[i, rows, :] = y[:, i * 128:(i + 1) * 128]
                qkv[5 + i, rows, :] = y[:, 512 + i * 128:512 + (i + 1) * 128]
                qkv[10 + i, rows, :] = y[:, 1024 + i * 128:1024 + (i + 1) * 128]
            t12 = y[:, 1536:1664]
            qkv[4, rows, :] = jnp.where(lane < 64, t12, 0.0)
            qkv[9, rows, :] = pltpu.roll(t12, 64, 1)
            qkv[14, rows, :] = y[:, 1664:1792]
            yield
            for g in range(T // R):
                base = HALO + r0 + g * R
                q = [qkv[i, pl.ds(base, R), :] for i in range(5)]
                ls = []
                for j in range(W):
                    s = None
                    for i in range(5):
                        t = q[i] * qkv[5 + i, pl.ds(base - 2 * j, R), :]
                        s = t if s is None else s + t
                    s = s + pltpu.roll(s, 64, 1)
                    s = s + pltpu.roll(s, 32, 1)
                    s = s * SCALE
                    if j > 0 and g == 0:
                        pos = r0 + jax.lax.broadcasted_iota(jnp.int32, (R, 128), 0)
                        s = jnp.where(pos >= 2 * j, s, -1e9)
                    ls.append(s)
                m = functools.reduce(jnp.maximum, ls)
                es = [jnp.exp(l - m) for l in ls]
                inv = 1.0 / functools.reduce(lambda a, b: a + b, es)
                for i in range(5):
                    o = None
                    for j in range(W):
                        t = es[j] * qkv[10 + i, pl.ds(base - 2 * j, R), :]
                        o = t if o is None else o + t
                    obuf[pl.ds(g * R, R), pl.ds(i * 128, 128)] = (o * inv).astype(bf16)
                yield
            if first_wo:
                relayout_wo()
            a = jax.lax.dot_general(woT[...], obuf[...], NT_DIMS, preferred_element_type=f32)
            x2 = xres[:, pl.ds(r0, T)] + a
            xres[:, pl.ds(r0, T)] = x2
            yield
            xhat[pl.ds(r0, T), :] = _ln_t(x2).astype(bf16).T
            yield

        def stage_f(r0):
            xh = xhat[pl.ds(r0, T), :]
            acc = None
            for c in range(NC):
                cs = pl.ds(c * FC, FC)
                g = jnp.dot(xh, wg[:, cs], preferred_element_type=f32)
                u = jnp.dot(xh, wu[:, cs], preferred_element_type=f32)
                h = (_gelu(g) * u).astype(bf16)
                t = jax.lax.dot_general(wdT[:, cs], h, NT_DIMS, preferred_element_type=f32)
                acc = t if acc is None else acc + t
                yield
            x3 = xres[:, pl.ds(r0, T)] + acc
            xres[:, pl.ds(r0, T)] = x3
            outbuf[:, pl.ds(r0, T)] = x3.astype(bf16)
            yield

        def run(*gens, pattern=None):
            gens = list(gens)
            alive = [True] * len(gens)
            k = 0
            if pattern is not None:
                for ch in pattern:
                    i = int(ch)
                    if alive[i]:
                        try:
                            next(gens[i])
                        except StopIteration:
                            alive[i] = False
            while any(alive):
                for i, g in enumerate(gens):
                    if alive[i]:
                        try:
                            next(g)
                        except StopIteration:
                            alive[i] = False

        for b in range(KA):
            load_x(b)
            run(stage_a(b * T, first_wo=(b == 0)))
        for b in range(KA, NB):
            load_x(b)
        cp_wg.wait(); cp_wu.wait(); cp_wd.wait()

        def slot(n, carry):
            rf = pl.multiple_of((n % NB) * T, T)
            ra = pl.multiple_of(((n + KA) % NB) * T, T)
            run(stage_f(rf), stage_a(ra), pattern=order)
            @pl.when(n >= NB)
            def _():
                cp_out(rf).start()
            return carry
        jax.lax.fori_loop(0, 2 * NB - KA, slot, 0)

        def slot_f(n, carry):
            rf = pl.multiple_of((n % NB) * T, T)
            run(stage_f(rf))
            @pl.when(n >= NB)
            def _():
                cp_out(rf).start()
            return carry
        jax.lax.fori_loop(2 * NB - KA, 2 * NB, slot_f, 0)
        for b in range(NB):
            cp_out(b * T).wait()

    @jax.jit
    def fn(A_x, A_wqkv, A_wo, B_x, B_w_gate, B_w_up, B_w_down):
        xT = jnp.transpose(A_x.reshape(S, D))
        wdT = jnp.transpose(B_w_down)
        hbm = pl.BlockSpec(memory_space=pltpu.HBM)
        outT = pl.pallas_call(
            kernel,
            out_shape=jax.ShapeDtypeStruct((D, S), bf16),
            in_specs=[hbm] * 6,
            out_specs=hbm,
            scratch_shapes=[
                pltpu.VMEM((D, S), bf16),
                pltpu.VMEM((D, S), f32),
                pltpu.VMEM((D, 3 * D), bf16),
                pltpu.VMEM((D, D), bf16),
                pltpu.VMEM((5, 3 * D, 128), f32),
                pltpu.VMEM((1792, D), bf16),
                pltpu.VMEM((D, 640), bf16),
                pltpu.VMEM((D, F), bf16),
                pltpu.VMEM((D, F), bf16),
                pltpu.VMEM((D, F), bf16),
                pltpu.VMEM((15, HALO + S, 128), f32),
                pltpu.VMEM((T, 640), bf16),
                pltpu.VMEM((S, D), bf16),
                pltpu.VMEM((D, S), bf16),
                pltpu.SemaphoreType.DMA((NB + 6,)),
            ],
            compiler_params=pltpu.CompilerParams(vmem_limit_bytes=120 * 1024 * 1024),
        )(xT, A_wqkv, A_wo, B_w_gate, B_w_up, wdT)
        return jnp.transpose(outT).reshape(1, S, D)
    return fn


pallas_interleave_layers__sliding_local_dilated__glu_gated_geglu__prompt_kernel = build()
```

```python
import functools
import numpy as np
import jax
import jax.numpy as jnp
import jax.experimental.pallas as pl
import jax.experimental.pallas.tpu as pltpu

S, D, F = 2048, 576, 4608
H, DH, W = 32, 18, 8
EPS = 1e-5
SCALE = DH ** -0.5
C0 = 0.7978845608028654
HALO = 16
XO = 1792
KP = 640
NT_DIMS = (((1,), (1,)), ((), ()))
f32, bf16 = jnp.float32, jnp.bfloat16


def _gelu(g):
    return 0.5 * g * (1.0 + jnp.tanh(C0 * (g + 0.044715 * (g * g * g))))


def _ln_t(x):
    m = jnp.mean(x, axis=0, keepdims=True)
    xc = x - m
    v = jnp.mean(xc * xc, axis=0, keepdims=True)
    return xc * jax.lax.rsqrt(v + EPS)


def _cat(xs):
    return xs[0] if len(xs) == 1 else jnp.concatenate(xs, axis=1)


DEF_SLOT = "g0 g1 d0 g2 d1 g3 d2 g4 d3 g5 d4 g6 d5 g7 d6 l1 A wo hc qm l2 g8 d7 d8 fin".split()
DEF_PRO = "l1 qa A wo hc cp qb l2 qc".split()


def build(T=256, FC=512, FCE=512, KA=6, R=8, slot_order=None, pro_order=None, QSP=6, QS2=10, NE=3, RP=64, chain_p=False, scopes=True, flags=None):
    NB = S // T
    NC = F // FC
    NT_C = FC // 128
    slot_order = slot_order or DEF_SLOT
    pro_order = pro_order or DEF_PRO
    if isinstance(slot_order, str): slot_order = slot_order.split()
    if isinstance(pro_order, str): pro_order = pro_order.split()

    def scope(name):
        import contextlib
        return jax.named_scope(name) if scopes else contextlib.nullcontext()

    def kernel(xT_hbm, wqkv_hbm, wo_hbm, wg_hbm, wu_hbm, wdT_hbm, outT_hbm,
               xin, xres, wqkv_raw, wo_raw, tmp, wx, woT, wg, wu, wdT,
               qcur, qnew, outbuf, sems):
        def cp_x(r0):
            return pltpu.make_async_copy(xT_hbm.at[:, pl.ds(r0, T)], xin.at[:, pl.ds(r0, T)], sems.at[r0 // T])
        def cp_wqkv(c, n):
            rows = pl.ds(pl.multiple_of(c * 128, 64), n)
            return pltpu.make_async_copy(wqkv_hbm.at[rows, :], wqkv_raw.at[rows, :], sems.at[NB + 6 + c])
        cp_wo = pltpu.make_async_copy(wo_hbm, wo_raw, sems.at[NB + 1])
        cp_ffn = [pltpu.make_async_copy(src, dst, sems.at[NB + 2 + k])
                  for k, (src, dst) in enumerate(((wg_hbm, wg), (wu_hbm, wu), (wdT_hbm, wdT)))]
        def cp_out(r0):
            return pltpu.make_async_copy(outbuf.at[:, pl.ds(r0, T)], outT_hbm.at[:, pl.ds(r0, T)], sems.at[NB + 5])

        cp_x(0).start()
        cp_wqkv(4, 64).start()
        for c in range(4):
            cp_wqkv(c, 128).start()
        cp_wo.start()

        qcur[pl.ds(0, 15), pl.ds(T, HALO), :] = jnp.zeros((15, HALO, 128), f32)
        wqkv_raw[pl.ds(D, KP - D), :] = jnp.zeros((KP - D, 3 * D), bf16)
        wx[:, pl.ds(3 * D, 64), :] = jnp.zeros((5, 64, 128), bf16)

        def load_x(r0):
            cp_x(r0).wait()
            xres[:, pl.ds(r0, T)] = xin[:, pl.ds(r0, T)].astype(f32)

        with scope("relayout"):
            cp_wqkv(4, 64).wait()
            def tr_c(i, carry):
                c = (i + 4) % 5
                @pl.when(i > 0)
                def _():
                    cp_wqkv(c, 128).wait()
                tmp[0] = wqkv_raw[pl.ds(pl.multiple_of(c * 128, 128), 128), :].astype(f32).T
                for p in range(3):
                    for d in range(DH):
                        row = p * 512 + d * 32 if d < 16 else 1536 + p * 64 + (d - 16) * 32
                        wx[c, pl.ds(row, H), :] = tmp[0, pl.ds(p * D + d, H, stride=DH), :].astype(bf16)
                return carry
            jax.lax.fori_loop(0, 5, tr_c, 0)
        for b in range(1, NB):
            cp_x(b * T).start()
        for cp in cp_ffn:
            cp.start()

        def relayout_wo():
            cp_wo.wait()
            for c in range(5):
                n = 128 if c < 4 else 64
                tmp[c, pl.ds(0, D), pl.ds(0, n)] = wo_raw[:, pl.ds(c * 128, n)].astype(f32)
            tmp[4, pl.ds(0, D), pl.ds(64, 64)] = jnp.zeros((D, 64), f32)
            for c in range(5):
                rows = jnp.concatenate([tmp[c, pl.ds(d, H, stride=DH), :] for d in range(DH)]
                                       + [jnp.zeros((KP - D, 128), f32)], axis=0)
                wt = rows.astype(bf16).T
                for k in range(5):
                    woT[k, pl.ds(c * 128, 128), :] = wt[:, k * 128:(k + 1) * 128]

        lane = jax.lax.broadcasted_iota(jnp.int32, (T, 128), 1)

        def ln_tok(x):
            xh = _ln_t(x).astype(bf16)
            return jnp.concatenate([xh, jnp.zeros((KP - D, T), bf16)], axis=0).T

        def pieces_qkv(r0, split=None, split2=None):
            QS = split
            st = {}
            def l1():
                x = xres[:, pl.ds(r0, T)]
                st["xh"] = ln_tok(x)
            def put(direct, i, val):
                if direct:
                    qcur[i, pl.ds(HALO, T), :] = val
                else:
                    qnew[i] = val
            def qm_part(t0, t1, direct):
                wp = _cat([wx[k, pl.ds(t0 * 128, (t1 - t0) * 128), :] for k in range(5)])
                y = jax.lax.dot_general(st["xh"], wp, NT_DIMS, preferred_element_type=f32)
                for t in range(t0, t1):
                    yt = y[:, (t - t0) * 128:(t - t0 + 1) * 128]
                    if t < 12:
                        put(direct, 5 * (t // 4) + t % 4, yt)
                    elif t == 12:
                        put(direct, 4, jnp.where(lane < 64, yt, 0.0))
                        put(direct, 9, pltpu.roll(yt, 64, 1))
                    else:
                        put(direct, 14, yt)
            def slots(t0, t1):
                r = []
                for t in range(t0, t1):
                    r += [5 * (t // 4) + t % 4] if t < 12 else ([4, 9] if t == 12 else [14])
                return r
            def hc():
                for i in range(5, 15):
                    qcur[i, pl.ds(0, HALO), :] = qcur[i, pl.ds(T, HALO), :]
            def cp():
                for i in slots(0, QS):
                    qcur[i, pl.ds(HALO, T), :] = qnew[i]
            if QS is None:
                return {"l1": l1, "hc": hc, "qm": lambda: qm_part(0, 14, True)}
            return {"l1": l1, "hc": hc, "qa": lambda: qm_part(0, QS, False), "qb": lambda: qm_part(QS, split2, True), "cp": cp, **({"qc": lambda: qm_part(split2, 14, True)} if split2 < 14 else {})}

        def pieces_att(r0, z, R):
            st = {}
            def grp(g):
                base = HALO + g * R
                q = [qcur[i, pl.ds(base, R), :] for i in range(5)]
                ls = []
                for j in range(W):
                    s = None
                    for i in range(5):
                        t = q[i] * qcur[5 + i, pl.ds(base - 2 * j, R), :]
                        s = t if s is None else s + t
                    s = s + pltpu.roll(s, 64, 1)
                    s = s + pltpu.roll(s, 32, 1)
                    s = s * SCALE
                    if j > 0 and g * R < 2 * j:
                        pos = (r0 + g * R) + jax.lax.broadcasted_iota(jnp.int32, (R, 128), 0)
                        s = jnp.where(pos >= 2 * j, s, -1e9)
                    ls.append(s)
                m = functools.reduce(jnp.maximum, ls)
                es = [jnp.exp(l - m) for l in ls]
                inv = 1.0 / functools.reduce(lambda a, b: a + b, es)
                for i in range(5):
                    o = None
                    for j in range(W):
                        t = es[j] * qcur[10 + i, pl.ds(base - 2 * j, R), :]
                        o = t if o is None else o + t
                    qcur[15 + i, pl.ds(pl.multiple_of(z + g * R, 8), R), :] = o * inv
            def wo():
                o = _cat([qcur[15 + k, pl.ds(pl.multiple_of(z, 8), T), :].astype(bf16) for k in range(5)])
                w = _cat([woT[k, pl.ds(0, D), :] for k in range(5)])
                a = jax.lax.dot_general(w, o, NT_DIMS, preferred_element_type=f32)
                x2 = xres[:, pl.ds(r0, T)] + a
                xres[:, pl.ds(r0, T)] = x2
                st["x2"] = x2
            def l2():
                xh = ln_tok(st["x2"])
                for k in range(5):
                    wx[k, pl.ds(XO + r0, T), :] = xh[:, k * 128:(k + 1) * 128]
            d = {f"a{g}": functools.partial(grp, g) for g in range(T // R)}
            d.update(wo=wo, l2=l2)
            return d

        def pieces_f(r0, c0, nc, fc, first=True, last=True):
            st = {}
            ntc = fc // 128
            def ldx():
                st["xh"] = _cat([wx[k, pl.ds(XO + r0, T), :] for k in range(4)] + [wx[4, pl.ds(XO + r0, T), pl.ds(0, 64)]])
                st["acc"] = xres[:, pl.ds(r0, T)]
            def gu(c):
                if "xh" not in st: ldx()
                cs = pl.ds(pl.multiple_of((c0 + c) * fc, 128), fc)
                g = jnp.dot(st["xh"], wg[:, cs], preferred_element_type=f32)
                u = jnp.dot(st["xh"], wu[:, cs], preferred_element_type=f32)
                st[c] = (_gelu(g) * u).astype(bf16)
            def dn(c):
                w = wdT[:, pl.ds(pl.multiple_of((c0 + c) * fc, 128), fc)]
                st["acc"] = st["acc"] + jax.lax.dot_general(w, st.pop(c), NT_DIMS, preferred_element_type=f32)
            def fin():
                xres[:, pl.ds(r0, T)] = st["acc"]
                outbuf[:, pl.ds(r0, T)] = st["acc"].astype(bf16)
            d = {}
            for c in range(nc):
                d[f"g{c}"] = functools.partial(gu, c)
                d[f"d{c}"] = functools.partial(dn, c)
            d["fin"] = fin
            return d

        def run(order, *piece_dicts):
            allp = {}
            for p in piece_dicts:
                allp.update(p)
            done = set()
            groups = [[]]
            for name in order:
                if name == "|":
                    groups.append([])
                else:
                    groups[-1].append(name)
            import contextlib
            for gi, grp in enumerate(groups):
                with (jax.named_scope(f"grp{gi}") if len(groups) > 1 else contextlib.nullcontext()):
                    for name in grp:
                        if name == "A":
                            for k in sorted((k for k in allp if k[0] == "a"), key=lambda k: int(k[1:])):
                                if k not in done:
                                    allp[k](); done.add(k)
                        if name in allp and name not in done:
                            allp[name]()
                            done.add(name)
            missing = set(allp) - done
            assert not missing, missing

        def blk(a):
            return pl.multiple_of((a % NB) * T, T)

        with scope("pro0"):
            load_x(0)
            run(["l1", "hc", "qm"], pieces_qkv(0))
            relayout_wo()
        def pro(a, c):
            load_x(blk(a + 1))
            run(pro_order, pieces_att(blk(a), (a // 64) * 8 if chain_p else 0, RP), pieces_qkv(blk(a + 1), QSP, QS2))
            return c
        with scope("pro_loop"):
            jax.lax.fori_loop(0, KA, pro, 0)
        with scope("w_ffn"):
            def lx(b, c):
                load_x(blk(b))
                return c
            jax.lax.fori_loop(KA + 1, NB, lx, 0)
            for cp in cp_ffn:
                cp.wait()

        def slot(n, carry):
            run(slot_order, pieces_f(blk(n), 0, NC, FC), pieces_att(blk(n + KA), (n // 64) * 8, R), pieces_qkv(blk(n + KA + 1)))
            @pl.when(n >= NB)
            def _():
                cp_out(blk(n)).start()
            return carry
        with scope("loop_fa"):
            jax.lax.fori_loop(0, 2 * NB - KA, slot, 0)

        NCE = F // NE // FCE
        e_order = ["g0"] + [x for c in range(1, NCE) for x in (f"g{c}", f"d{c-1}")] + [f"d{NCE-1}", "fin"]
        def slot_f(m, carry):
            n = m // NE
            hf = m % NE
            run(e_order, pieces_f(blk(n), hf * NCE, NCE, FCE))
            @pl.when(hf == NE - 1)
            def _():
                cp_out(blk(n)).start()
            return carry
        with scope("loop_f"):
            jax.lax.fori_loop(NE * (2 * NB - KA), NE * 2 * NB, slot_f, 0)
        with scope("w_out"):
            for b in range(NB):
                cp_out(b * T).wait()

    @jax.jit
    def fn(A_x, A_wqkv, A_wo, B_x, B_w_gate, B_w_up, B_w_down):
        xT = jnp.transpose(A_x.reshape(S, D))
        wdT = jnp.transpose(B_w_down)
        hbm = pl.BlockSpec(memory_space=pltpu.HBM)
        outT = pl.pallas_call(
            kernel,
            out_shape=jax.ShapeDtypeStruct((D, S), bf16),
            in_specs=[hbm] * 6,
            out_specs=hbm,
            scratch_shapes=[
                pltpu.VMEM((D, S), bf16),
                pltpu.VMEM((D, S), f32),
                pltpu.VMEM((KP, 3 * D), bf16),
                pltpu.VMEM((D, D), bf16),
                pltpu.VMEM((5, 3 * D, 128), f32),
                pltpu.VMEM((5, 1792 + S, 128), bf16),
                pltpu.VMEM((5, KP, 128), bf16),
                pltpu.VMEM((D, F), bf16),
                pltpu.VMEM((D, F), bf16),
                pltpu.VMEM((D, F), bf16),
                pltpu.VMEM((20, HALO + T, 128), f32),
                pltpu.VMEM((15, T, 128), f32),
                pltpu.VMEM((D, S), bf16),
                pltpu.SemaphoreType.DMA((NB + 11,)),
            ],
            compiler_params=pltpu.CompilerParams(vmem_limit_bytes=120 * 1024 * 1024, flags=flags) if flags else pltpu.CompilerParams(vmem_limit_bytes=120 * 1024 * 1024),
        )(xT, A_wqkv, A_wo, B_w_gate, B_w_up, wdT)
        return jnp.transpose(outT).reshape(1, S, D)
    return fn


pallas_interleave_layers__sliding_local_dilated__glu_gated_geglu__prompt_kernel = build(KA=4, scopes=False, flags={'XLA_TPU_FORCE_LP_LLO_SCHEDULER': True})
```

```python
import functools
import numpy as np
import jax
import jax.numpy as jnp
import jax.experimental.pallas as pl
import jax.experimental.pallas.tpu as pltpu

S, D, F = 2048, 576, 4608
H, DH, W = 32, 18, 8
EPS = 1e-5
SCALE = DH ** -0.5
C0 = 0.7978845608028654
HALO = 16
XO = 1792
KP = 640
NT_DIMS = (((1,), (1,)), ((), ()))
f32, bf16 = jnp.float32, jnp.bfloat16


def _gelu(g):
    return 0.5 * g * (1.0 + jnp.tanh(C0 * (g + 0.044715 * (g * g * g))))


def _ln_t(x):
    m = jnp.mean(x, axis=0, keepdims=True)
    xc = x - m
    v = jnp.mean(xc * xc, axis=0, keepdims=True)
    return xc * jax.lax.rsqrt(v + EPS)


def _cat(xs):
    return xs[0] if len(xs) == 1 else jnp.concatenate(xs, axis=1)


DEF_SLOT = "g0 l1 hc qm g1 d0 g2 d1 g3 d2 g4 d3 g5 d4 g6 d5 g7 d6 A wo l2 g8 d7 d8 fin".split()
DEF_PRO = "l1 qa A wo hc cp qb l2 qc".split()


def build(T=256, FC=512, FCE=512, KA=1, R=8, slot_order=None, pro_order=None, QSP=6, QS2=10, NE=3, RP=64, chain_p=False, skew=0, WG=(0, 3, 6, 9), phased=True, early=True, dma_order='x1 w0 w1 w2 x2 x3 x4 x5 x6 x7', scopes=True, flags=None):
    NB = S // T
    WG = list(WG)
    NC = F // FC
    NT_C = FC // 128
    slot_order = slot_order or DEF_SLOT
    pro_order = pro_order or DEF_PRO
    if isinstance(slot_order, str): slot_order = slot_order.split()
    if isinstance(pro_order, str): pro_order = pro_order.split()

    def scope(name):
        import contextlib
        return jax.named_scope(name) if scopes else contextlib.nullcontext()

    def kernel(xT_hbm, wqkv_hbm, wo_hbm, wg_hbm, wu_hbm, wdT_hbm, outT_hbm,
               xin, xres, wqkv_raw, wo_raw, tmp, wx, woT, wg, wu, wdT,
               qcur, qnew, outbuf, sems):
        def cp_x(r0):
            return pltpu.make_async_copy(xT_hbm.at[:, pl.ds(r0, T)], xin.at[:, pl.ds(r0, T)], sems.at[r0 // T])
        def cp_wqkv(c, n):
            rows = pl.ds(pl.multiple_of(c * 128, 64), n)
            return pltpu.make_async_copy(wqkv_hbm.at[rows, :], wqkv_raw.at[rows, :], sems.at[NB + 6 + c])
        cp_wo = pltpu.make_async_copy(wo_hbm, wo_raw, sems.at[NB + 1])
        def cp_ffn(gi):
            c0, c1 = WG[gi], WG[gi + 1]
            cs = pl.ds(c0 * FC, (c1 - c0) * FC)
            return [pltpu.make_async_copy(src.at[:, cs], dst.at[:, cs], sems.at[NB + 11 + gi])
                    for src, dst in ((wg_hbm, wg), (wu_hbm, wu), (wdT_hbm, wdT))]
        def cp_out(r0):
            return pltpu.make_async_copy(outbuf.at[:, pl.ds(r0, T)], outT_hbm.at[:, pl.ds(r0, T)], sems.at[NB + 5])

        cp_x(0).start()
        cp_wqkv(4, 64).start()
        for c in range(4):
            cp_wqkv(c, 128).start()
        cp_wo.start()

        qcur[pl.ds(0, 15), pl.ds(T, HALO), :] = jnp.zeros((15, HALO, 128), f32)
        wqkv_raw[pl.ds(D, KP - D), :] = jnp.zeros((KP - D, 3 * D), bf16)
        wx[:, pl.ds(3 * D, 64), :] = jnp.zeros((5, 64, 128), bf16)

        def load_x(r0):
            cp_x(r0).wait()
            xres[:, pl.ds(r0, T)] = xin[:, pl.ds(r0, T)].astype(f32)

        def getx(r0, first):
            if first is None:
                return xres[:, pl.ds(r0, T)]
            return jnp.where(first, xin[:, pl.ds(r0, T)].astype(f32), xres[:, pl.ds(r0, T)])

        def ln_tok(x):
            xh = _ln_t(x).astype(bf16)
            return jnp.concatenate([xh, jnp.zeros((KP - D, T), bf16)], axis=0).T

        def relayout_wo():
            cp_wo.wait()
            for c in range(5):
                n = 128 if c < 4 else 64
                tmp[c, pl.ds(0, D), pl.ds(0, n)] = wo_raw[:, pl.ds(c * 128, n)].astype(f32)
            tmp[4, pl.ds(0, D), pl.ds(64, 64)] = jnp.zeros((D, 64), f32)
            for c in range(5):
                yield
                rows = jnp.concatenate([tmp[c, pl.ds(d, H, stride=DH), :] for d in range(DH)]
                                       + [jnp.zeros((KP - D, 128), f32)], axis=0)
                wt = rows.astype(bf16).T
                for k in range(5):
                    woT[k, pl.ds(c * 128, 128), :] = wt[:, k * 128:(k + 1) * 128]

        if early:
            load_x(0)
            xh0 = ln_tok(xres[:, pl.ds(0, T)])
            for k in range(5):
                wx[k, pl.ds(XO, T), :] = xh0[:, k * 128:(k + 1) * 128]

        with scope("relayout"):
            cp_wqkv(4, 64).wait()
            def tr_c(i, carry):
                c = (i + 4) % 5
                @pl.when(i > 0)
                def _():
                    cp_wqkv(c, 128).wait()
                tmp[0] = wqkv_raw[pl.ds(pl.multiple_of(c * 128, 128), 128), :].astype(f32).T
                for p in range(3):
                    for d in range(DH):
                        row = p * 512 + d * 32 if d < 16 else 1536 + p * 64 + (d - 16) * 32
                        wx[c, pl.ds(row, H), :] = tmp[0, pl.ds(p * D + d, H, stride=DH), :].astype(bf16)
                return carry
            jax.lax.fori_loop(0, 5, tr_c, 0)
        for item in dma_order.split():
            if item[0] == "x":
                cp_x(int(item[1:]) * T).start()
            else:
                for cp in cp_ffn(int(item[1:])):
                    cp.start()

        lane = jax.lax.broadcasted_iota(jnp.int32, (T, 128), 1)

        def pieces_qkv(r0, split=None, split2=None, first=None, pre=False):
            QS = split
            st = {}
            def l1():
                if pre:
                    st["xh"] = _cat([wx[k, pl.ds(XO, T), :] for k in range(5)])
                else:
                    st["xh"] = ln_tok(getx(r0, first))
            def put(direct, i, val):
                if direct:
                    qcur[i, pl.ds(HALO, T), :] = val
                else:
                    qnew[i] = val
            def qm_part(t0, t1, direct):
                wp = _cat([wx[k, pl.ds(t0 * 128, (t1 - t0) * 128), :] for k in range(5)])
                y = jax.lax.dot_general(st["xh"], wp, NT_DIMS, preferred_element_type=f32)
                for t in range(t0, t1):
                    yt = y[:, (t - t0) * 128:(t - t0 + 1) * 128]
                    if t < 12:
                        put(direct, 5 * (t // 4) + t % 4, yt)
                    elif t == 12:
                        put(direct, 4, jnp.where(lane < 64, yt, 0.0))
                        put(direct, 9, pltpu.roll(yt, 64, 1))
                    else:
                        put(direct, 14, yt)
            def slots(t0, t1):
                r = []
                for t in range(t0, t1):
                    r += [5 * (t // 4) + t % 4] if t < 12 else ([4, 9] if t == 12 else [14])
                return r
            def hc():
                for i in range(5, 15):
                    qcur[i, pl.ds(0, HALO), :] = qcur[i, pl.ds(T, HALO), :]
            def cp():
                for i in slots(0, QS):
                    qcur[i, pl.ds(HALO, T), :] = qnew[i]
            if QS is None:
                return {"l1": l1, "hc": hc, "qm": lambda: qm_part(0, 14, True), **({"part": qm_part} if pre else {})}
            return {"l1": l1, "hc": hc, "qa": lambda: qm_part(0, QS, False), "qb": lambda: qm_part(QS, split2, True), "cp": cp, **({"qc": lambda: qm_part(split2, 14, True)} if split2 < 14 else {})}

        def pieces_att(r0, z, R, first=None):
            st = {}
            def grp(g):
                base = HALO + g * R
                q = [qcur[i, pl.ds(base, R), :] for i in range(5)]
                ls = []
                for j in range(W):
                    s = None
                    for i in range(5):
                        t = q[i] * qcur[5 + i, pl.ds(base - 2 * j, R), :]
                        s = t if s is None else s + t
                    s = s + pltpu.roll(s, 64, 1)
                    s = s + pltpu.roll(s, 32, 1)
                    s = s * SCALE
                    if j > 0 and g * R < 2 * j:
                        pos = (r0 + g * R) + jax.lax.broadcasted_iota(jnp.int32, (R, 128), 0)
                        s = jnp.where(pos >= 2 * j, s, -1e9)
                    ls.append(s)
                m = functools.reduce(jnp.maximum, ls)
                es = [jnp.exp(l - m) for l in ls]
                inv = 1.0 / functools.reduce(lambda a, b: a + b, es)
                for i in range(5):
                    o = None
                    for j in range(W):
                        t = es[j] * qcur[10 + i, pl.ds(base - 2 * j, R), :]
                        o = t if o is None else o + t
                    qcur[15 + i, pl.ds(pl.multiple_of(z + g * R, 8), R), :] = o * inv
            def wo():
                o = _cat([qcur[15 + k, pl.ds(pl.multiple_of(z, 8), T), :].astype(bf16) for k in range(5)])
                w = _cat([woT[k, pl.ds(0, D), :] for k in range(5)])
                a = jax.lax.dot_general(w, o, NT_DIMS, preferred_element_type=f32)
                x2 = getx(r0, first) + a
                xres[:, pl.ds(r0, T)] = x2
                st["x2"] = x2
            def l2():
                xh = ln_tok(st["x2"])
                for k in range(5):
                    wx[k, pl.ds(XO + r0, T), :] = xh[:, k * 128:(k + 1) * 128]
            d = {f"a{g}": functools.partial(grp, g) for g in range(T // R)}
            d.update(wo=wo, l2=l2)
            return d

        def pieces_f(r0, c0, nc, fc, first=True, last=True):
            st = {}
            ntc = fc // 128
            def ldx():
                st["xh"] = _cat([wx[k, pl.ds(XO + r0, T), :] for k in range(4)] + [wx[4, pl.ds(XO + r0, T), pl.ds(0, 64)]])
                st["acc"] = xres[:, pl.ds(r0, T)]
            def gu(c):
                if "xh" not in st: ldx()
                cs = pl.ds(pl.multiple_of((c0 + c) * fc, 128), fc)
                g = jnp.dot(st["xh"], wg[:, cs], preferred_element_type=f32)
                u = jnp.dot(st["xh"], wu[:, cs], preferred_element_type=f32)
                st[c] = (_gelu(g) * u).astype(bf16)
            def dn(c):
                w = wdT[:, pl.ds(pl.multiple_of((c0 + c) * fc, 128), fc)]
                st["acc"] = st["acc"] + jax.lax.dot_general(w, st.pop(c), NT_DIMS, preferred_element_type=f32)
            def fin():
                xres[:, pl.ds(r0, T)] = st["acc"]
                outbuf[:, pl.ds(r0, T)] = st["acc"].astype(bf16)
            d = {}
            for c in range(nc):
                d[f"g{c}"] = functools.partial(gu, c)
                d[f"d{c}"] = functools.partial(dn, c)
            d["fin"] = fin
            return d

        def run(order, *piece_dicts):
            allp = {}
            for p in piece_dicts:
                allp.update(p)
            done = set()
            groups = [[]]
            for name in order:
                if name == "|":
                    groups.append([])
                else:
                    groups[-1].append(name)
            import contextlib
            for gi, grp in enumerate(groups):
                with (jax.named_scope(f"grp{gi}") if len(groups) > 1 else contextlib.nullcontext()):
                    for name in grp:
                        if name == "A":
                            for k in sorted((k for k in allp if k[0] == "a"), key=lambda k: int(k[1:])):
                                if k not in done:
                                    allp[k](); done.add(k)
                        if name in allp and name not in done:
                            allp[name]()
                            done.add(name)
            missing = set(allp) - done
            assert not missing, missing

        def blk(a):
            return pl.multiple_of((a % NB) * T, T)

        with scope("pro0"):
            if early:
                pq = pieces_qkv(0, pre=True)
                pq["l1"](); pq["hc"]()
                rw = relayout_wo()
                bounds = (0, 2, 4, 7, 10, 12, 14)
                for i in range(6):
                    pq["part"](bounds[i], bounds[i + 1], True)
                    next(rw, None)
            else:
                load_x(0)
                run(["l1", "hc", "qm", "part"], {**pieces_qkv(0), "part": lambda: None})
                for _ in relayout_wo():
                    pass
        def pro(a, c):
            load_x(blk(a + 1))
            run(pro_order, pieces_att(blk(a), (a // 64) * 8 if chain_p else 0, RP), pieces_qkv(blk(a + 1), QSP, QS2))
            return c
        with scope("pro_loop"):
            NP = KA + 1 if phased else KA
            jax.lax.fori_loop(0, NP - 1 + skew, pro, 0)
            if not skew:
                run("A wo l2".split(), pieces_att((NP - 1) * T, 0, RP))
        def wx_(b, c):
            cp_x(blk(b)).wait()
            return c
        def lx(b, c):
            load_x(blk(b))
            return c
        if not phased:
            with scope("w_ffn"):
                jax.lax.fori_loop(KA + skew, NB, lx, 0)
                for gi in range(len(WG) - 1):
                    for cp in cp_ffn(gi):
                        cp.wait()

        def slot(n, carry):
            run(slot_order, pieces_f(blk(n), 0, NC, FC), pieces_att(blk(n + KA), (n // 64) * 8, R, n + KA < NB), pieces_qkv(blk(n + KA + skew), first=n + KA + skew < NB))
            @pl.when(n >= NB)
            def _():
                cp_out(blk(n)).start()
            return carry
        NCE = F // NE // FCE
        e_order = ["g0"] + [x for c in range(1, NCE) for x in (f"g{c}", f"d{c-1}")] + [f"d{NCE-1}", "fin"]
        def slot_f(m, carry):
            n = m // NE
            hf = m % NE
            if phased:
                for gi in range(NE):
                    @pl.when(m == gi)
                    def _():
                        for cp in cp_ffn(gi):
                            cp.wait()
            run(e_order, pieces_f(blk(n), hf * NCE, NCE, FCE))
            @pl.when(jnp.logical_and(hf == NE - 1, n >= NB))
            def _():
                cp_out(blk(n)).start()
            return carry

        if phased:
            def phase(ph, carry):
                jax.lax.fori_loop(KA + 1, KA + 1 + ph * (NB - KA - 1), wx_, 0)
                with scope("loop_fa"):
                    jax.lax.fori_loop(1, 1 + ph * (2 * NB - KA - 1), slot, 0)
                with scope("loop_f"):
                    jax.lax.fori_loop(ph * NE * (2 * NB - KA), NE + ph * NE * (2 * NB - 1), slot_f, 0)
                return carry
            jax.lax.fori_loop(0, 2, phase, 0)
        else:
            with scope("loop_fa"):
                jax.lax.fori_loop(0, 2 * NB - KA, slot, 0)
            with scope("loop_f"):
                jax.lax.fori_loop(NE * (2 * NB - KA), NE * 2 * NB, slot_f, 0)
        with scope("w_out"):
            for b in range(NB):
                cp_out(b * T).wait()

    @jax.jit
    def fn(A_x, A_wqkv, A_wo, B_x, B_w_gate, B_w_up, B_w_down):
        xT = jnp.transpose(A_x.reshape(S, D))
        wdT = jnp.transpose(B_w_down)
        hbm = pl.BlockSpec(memory_space=pltpu.HBM)
        outT = pl.pallas_call(
            kernel,
            out_shape=jax.ShapeDtypeStruct((D, S), bf16),
            in_specs=[hbm] * 6,
            out_specs=hbm,
            scratch_shapes=[
                pltpu.VMEM((D, S), bf16),
                pltpu.VMEM((D, S), f32),
                pltpu.VMEM((KP, 3 * D), bf16),
                pltpu.VMEM((D, D), bf16),
                pltpu.VMEM((5, 3 * D, 128), f32),
                pltpu.VMEM((5, 1792 + S, 128), bf16),
                pltpu.VMEM((5, KP, 128), bf16),
                pltpu.VMEM((D, F), bf16),
                pltpu.VMEM((D, F), bf16),
                pltpu.VMEM((D, F), bf16),
                pltpu.VMEM((20, HALO + T, 128), f32),
                pltpu.VMEM((15, T, 128), f32),
                pltpu.VMEM((D, S), bf16),
                pltpu.SemaphoreType.DMA((NB + 11 + len(WG),)),
            ],
            compiler_params=pltpu.CompilerParams(vmem_limit_bytes=120 * 1024 * 1024, flags=flags) if flags else pltpu.CompilerParams(vmem_limit_bytes=120 * 1024 * 1024),
        )(xT, A_wqkv, A_wo, B_w_gate, B_w_up, wdT)
        return jnp.transpose(outT).reshape(1, S, D)
    return fn


pallas_interleave_layers__sliding_local_dilated__glu_gated_geglu__prompt_kernel = build(scopes=False, flags={'XLA_TPU_FORCE_LP_LLO_SCHEDULER': True})
```

```python
import functools

import jax
import jax.numpy as jnp
import jax.experimental.pallas as pl
import jax.experimental.pallas.tpu as pltpu

S, D, F = 2048, 576, 4608
H, DH, W, DIL = 32, 18, 8, 2
EPS = 1e-5
SCALE = DH ** -0.5
C0 = 0.7978845608028654
T = 256
NB = S // T
HALO = 16
KP = 640
NQ = 1792
FC = 512
NC = F // FC
NE = 3
QCOLS = (0, 640, 1152, 3 * D)
QS1, QS2 = 6, 10
NT_DIMS = (((1,), (1,)), ((), ()))
f32, bf16 = jnp.float32, jnp.bfloat16

SLOT_ORDER = "g0 l1 hc qm g1 d0 g2 d1 g3 d2 g4 d3 g5 d4 g6 d5 g7 d6 A wo l2 g8 d7 d8 fin".split()
PRO_ORDER = "l1 qa A wo hc cp qb l2 qc".split()


def _gelu(g):
    return 0.5 * g * (1.0 + jnp.tanh(C0 * (g + 0.044715 * (g * g * g))))


def _cat(xs):
    return jnp.concatenate(xs, axis=1)


def _ln_tok(x):
    m = jnp.mean(x, axis=0, keepdims=True)
    xc = x - m
    v = jnp.mean(xc * xc, axis=0, keepdims=True)
    xh = (xc * jax.lax.rsqrt(v + EPS)).astype(bf16)
    return jnp.concatenate([xh, jnp.zeros((KP - D, T), bf16)], axis=0).T


def _run(order, *piece_dicts):
    pieces = {}
    for p in piece_dicts:
        pieces.update(p)
    for name in order:
        if name == "A":
            g = 0
            while f"a{g}" in pieces:
                pieces.pop(f"a{g}")()
                g += 1
        else:
            pieces.pop(name)()
    assert not pieces


def _blk(a):
    return pl.multiple_of((a % NB) * T, T)


def _kernel(xT_hbm, wqkv_hbm, wo_hbm, wg_hbm, wu_hbm, wdT_hbm, outT_hbm,
            xin, xres, wqkv_raw, wo_raw, tmp, wx, woT, wg, wu, wdT, qcur, qnew, outbuf, sems):
    def cp_x(r0):
        return pltpu.make_async_copy(xT_hbm.at[:, pl.ds(r0, T)], xin.at[:, pl.ds(r0, T)], sems.at[r0 // T])

    def cp_out(r0):
        return pltpu.make_async_copy(outbuf.at[:, pl.ds(r0, T)], outT_hbm.at[:, pl.ds(r0, T)], sems.at[NB])

    cp_wo = pltpu.make_async_copy(wo_hbm, wo_raw, sems.at[NB + 1])

    def cp_wqkv(p):
        cols = pl.ds(QCOLS[p], QCOLS[p + 1] - QCOLS[p])
        return pltpu.make_async_copy(wqkv_hbm.at[:, cols], wqkv_raw.at[pl.ds(0, D), cols], sems.at[NB + 2 + p])

    def cp_ffn(part):
        cols = pl.ds(part * (F // NE), F // NE)
        return [pltpu.make_async_copy(src.at[:, cols], dst.at[:, cols], sems.at[NB + 5 + part])
                for src, dst in ((wg_hbm, wg), (wu_hbm, wu), (wdT_hbm, wdT))]

    def load_x(r0):
        cp_x(r0).wait()
        xres[:, pl.ds(r0, T)] = xin[:, pl.ds(r0, T)].astype(f32)

    def getx(r0, first):
        if first is None:
            return xres[:, pl.ds(r0, T)]
        return jnp.where(first, xin[:, pl.ds(r0, T)].astype(f32), xres[:, pl.ds(r0, T)])

    def relayout_qkv(p):
        cp_wqkv(p).wait()
        c0, c1 = QCOLS[p], QCOLS[p + 1]
        for c in range(5):
            tmp[c, pl.ds(c0, c1 - c0), :] = wqkv_raw[pl.ds(c * 128, 128), pl.ds(c0, c1 - c0)].astype(f32).T
        yield
        for c in range(5):
            for d in range(DH):
                row = p * 512 + d * 32 if d < 16 else 1536 + p * 64 + (d - 16) * 32
                wx[c, pl.ds(row, H), :] = tmp[c, pl.ds(p * D + d, H, stride=DH), :].astype(bf16)

    def relayout_wo():
        cp_wo.wait()
        for c in range(5):
            n = 128 if c < 4 else 64
            tmp[c, pl.ds(0, D), pl.ds(0, n)] = wo_raw[:, pl.ds(c * 128, n)].astype(f32)
        tmp[4, pl.ds(0, D), pl.ds(64, 64)] = jnp.zeros((D, 64), f32)
        for c in range(5):
            yield
            rows = jnp.concatenate([tmp[c, pl.ds(d, H, stride=DH), :] for d in range(DH)]
                                   + [jnp.zeros((KP - D, 128), f32)], axis=0)
            wt = rows.astype(bf16).T
            for k in range(5):
                woT[k, pl.ds(c * 128, 128), :] = wt[:, k * 128:(k + 1) * 128]

    lane = jax.lax.broadcasted_iota(jnp.int32, (T, 128), 1)

    def pieces_qkv(r0, first=None, split=False, pre=False):
        st = {}

        def l1():
            if pre:
                st["xh"] = _cat([wx[k, pl.ds(NQ, T), :] for k in range(5)])
            else:
                st["xh"] = _ln_tok(getx(r0, first))

        def put(direct, i, val):
            if direct:
                qcur[i, pl.ds(HALO, T), :] = val
            else:
                qnew[i] = val

        def part(t0, t1, direct=True):
            wp = _cat([wx[k, pl.ds(t0 * 128, (t1 - t0) * 128), :] for k in range(5)])
            y = jax.lax.dot_general(st["xh"], wp, NT_DIMS, preferred_element_type=f32)
            for t in range(t0, t1):
                yt = y[:, (t - t0) * 128:(t - t0 + 1) * 128]
                if t < 12:
                    put(direct, 5 * (t // 4) + t % 4, yt)
                elif t == 12:
                    put(direct, 4, jnp.where(lane < 64, yt, 0.0))
                    put(direct, 9, pltpu.roll(yt, 64, 1))
                else:
                    put(direct, 14, yt)

        def hc():
            for i in range(5, 15):
                qcur[i, pl.ds(0, HALO), :] = qcur[i, pl.ds(T, HALO), :]

        def cp():
            for i in range(QS1):
                qcur[5 * (i // 4) + i % 4, pl.ds(HALO, T), :] = qnew[5 * (i // 4) + i % 4]

        if split:
            return {"l1": l1, "hc": hc, "cp": cp, "qa": lambda: part(0, QS1, False),
                    "qb": lambda: part(QS1, QS2), "qc": lambda: part(QS2, 14)}
        if pre:
            return {"l1": l1, "hc": hc, "part": part}
        return {"l1": l1, "hc": hc, "qm": lambda: part(0, 14)}

    def pieces_att(r0, R, z=0, first=None):
        st = {}

        def grp(g):
            base = HALO + g * R
            q = [qcur[i, pl.ds(base, R), :] for i in range(5)]
            ls = []
            for j in range(W):
                s = None
                for i in range(5):
                    t = q[i] * qcur[5 + i, pl.ds(base - DIL * j, R), :]
                    s = t if s is None else s + t
                s = s + pltpu.roll(s, 64, 1)
                s = s + pltpu.roll(s, 32, 1)
                s = s * SCALE
                if j > 0 and g * R < DIL * j:
                    pos = (r0 + g * R) + jax.lax.broadcasted_iota(jnp.int32, (R, 128), 0)
                    s = jnp.where(pos >= DIL * j, s, -1e9)
                ls.append(s)
            m = functools.reduce(jnp.maximum, ls)
            es = [jnp.exp(l - m) for l in ls]
            inv = 1.0 / functools.reduce(lambda a, b: a + b, es)
            for i in range(5):
                o = None
                for j in range(W):
                    t = es[j] * qcur[10 + i, pl.ds(base - DIL * j, R), :]
                    o = t if o is None else o + t
                qcur[15 + i, pl.ds(pl.multiple_of(z + g * R, 8), R), :] = o * inv

        def wo():
            o = _cat([qcur[15 + k, pl.ds(pl.multiple_of(z, 8), T), :].astype(bf16) for k in range(5)])
            w = _cat([woT[k, pl.ds(0, D), :] for k in range(5)])
            a = jax.lax.dot_general(w, o, NT_DIMS, preferred_element_type=f32)
            x2 = getx(r0, first) + a
            xres[:, pl.ds(r0, T)] = x2
            st["x2"] = x2

        def l2():
            xh = _ln_tok(st["x2"])
            for k in range(5):
                wx[k, pl.ds(NQ + r0, T), :] = xh[:, k * 128:(k + 1) * 128]

        d = {f"a{g}": functools.partial(grp, g) for g in range(T // R)}
        d.update(wo=wo, l2=l2)
        return d

    def pieces_f(r0, c0, nc):
        st = {}

        def cols(c):
            return pl.ds(pl.multiple_of((c0 + c) * FC, 128), FC)

        def gu(c):
            if "xh" not in st:
                st["xh"] = _cat([wx[k, pl.ds(NQ + r0, T), :] for k in range(4)]
                                + [wx[4, pl.ds(NQ + r0, T), pl.ds(0, D - 512)]])
                st["acc"] = xres[:, pl.ds(r0, T)]
            g = jnp.dot(st["xh"], wg[:, cols(c)], preferred_element_type=f32)
            u = jnp.dot(st["xh"], wu[:, cols(c)], preferred_element_type=f32)
            st[c] = (_gelu(g) * u).astype(bf16)

        def dn(c):
            st["acc"] = st["acc"] + jax.lax.dot_general(
                wdT[:, cols(c)], st.pop(c), NT_DIMS, preferred_element_type=f32)

        def fin():
            xres[:, pl.ds(r0, T)] = st["acc"]
            outbuf[:, pl.ds(r0, T)] = st["acc"].astype(bf16)

        d = {"fin": fin}
        for c in range(nc):
            d[f"g{c}"] = functools.partial(gu, c)
            d[f"d{c}"] = functools.partial(dn, c)
        return d

    cp_x(0).start()
    for p in range(3):
        cp_wqkv(p).start()
    cp_wo.start()
    qcur[pl.ds(0, 15), pl.ds(T, HALO), :] = jnp.zeros((15, HALO, 128), f32)
    wqkv_raw[pl.ds(D, KP - D), :] = jnp.zeros((KP - D, 3 * D), bf16)
    wx[:, pl.ds(3 * D, NQ - 3 * D), :] = jnp.zeros((5, NQ - 3 * D, 128), bf16)

    load_x(0)
    xh0 = _ln_tok(xres[:, pl.ds(0, T)])
    for k in range(5):
        wx[k, pl.ds(NQ, T), :] = xh0[:, k * 128:(k + 1) * 128]

    pq = pieces_qkv(0, pre=True)
    pq["l1"]()
    pq["hc"]()
    rq, rk, rv, rw = relayout_qkv(0), relayout_qkv(1), relayout_qkv(2), relayout_wo()
    list(rq)
    next(rk)
    pq["part"](0, 4)
    list(rk)
    next(rv)
    cp_x(T).start()
    for p in range(NE):
        for cp in cp_ffn(p):
            cp.start()
    for b in range(2, NB):
        cp_x(b * T).start()
    pq["part"](4, 8)
    list(rv)
    next(rw)
    pq["part"](12, 13)
    next(rw)
    next(rw)
    pq["part"](8, 10)
    next(rw)
    next(rw)
    pq["part"](10, 12)
    list(rw)
    pq["part"](13, 14)

    load_x(T)
    _run(PRO_ORDER, pieces_att(0, 64), pieces_qkv(T, split=True))
    _run(["A", "wo", "l2"], pieces_att(T, 64))

    def slot(n, carry):
        first = n + 1 < NB
        _run(SLOT_ORDER, pieces_f(_blk(n), 0, NC),
             pieces_att(_blk(n + 1), 8, (n // 64) * 8, first), pieces_qkv(_blk(n + 1), first))

        @pl.when(n >= NB)
        def _():
            cp_out(_blk(n)).start()
        return carry

    nce = NC // NE
    e_order = ["g0"] + [x for c in range(1, nce) for x in (f"g{c}", f"d{c - 1}")] + [f"d{nce - 1}", "fin"]

    def slot_f(m, carry):
        n = m // NE
        part = m % NE
        for p in range(NE):
            @pl.when(m == p)
            def _():
                for cp in cp_ffn(p):
                    cp.wait()
        _run(e_order, pieces_f(_blk(n), part * nce, nce))

        @pl.when(jnp.logical_and(part == NE - 1, n >= NB))
        def _():
            cp_out(_blk(n)).start()
        return carry

    def wait_x(b, carry):
        cp_x(_blk(b)).wait()
        return carry

    def phase(ph, carry):
        jax.lax.fori_loop(2, 2 + ph * (NB - 2), wait_x, 0)
        jax.lax.fori_loop(1, 1 + ph * (2 * NB - 2), slot, 0)
        jax.lax.fori_loop(ph * NE * (2 * NB - 1), NE + ph * NE * (2 * NB - 1), slot_f, 0)
        return carry
    jax.lax.fori_loop(0, 2, phase, 0)
    for b in range(NB):
        cp_out(b * T).wait()


@jax.jit
def pallas_interleave_layers__sliding_local_dilated__glu_gated_geglu__prompt_kernel(
    A_x: jax.Array,
    A_wqkv: jax.Array,
    A_wo: jax.Array,
    B_x: jax.Array,
    B_w_gate: jax.Array,
    B_w_up: jax.Array,
    B_w_down: jax.Array,
):
    del B_x
    hbm = pl.BlockSpec(memory_space=pltpu.HBM)
    out_t = pl.pallas_call(
        _kernel,
        out_shape=jax.ShapeDtypeStruct((D, S), bf16),
        in_specs=[hbm] * 6,
        out_specs=hbm,
        scratch_shapes=[
            pltpu.VMEM((D, S), bf16),
            pltpu.VMEM((D, S), f32),
            pltpu.VMEM((KP, 3 * D), bf16),
            pltpu.VMEM((D, D), bf16),
            pltpu.VMEM((5, 3 * D, 128), f32),
            pltpu.VMEM((5, NQ + S, 128), bf16),
            pltpu.VMEM((5, KP, 128), bf16),
            pltpu.VMEM((D, F), bf16),
            pltpu.VMEM((D, F), bf16),
            pltpu.VMEM((D, F), bf16),
            pltpu.VMEM((20, HALO + T, 128), f32),
            pltpu.VMEM((15, T, 128), f32),
            pltpu.VMEM((D, S), bf16),
            pltpu.SemaphoreType.DMA((NB + 5 + NE,)),
        ],
        compiler_params=pltpu.CompilerParams(
            vmem_limit_bytes=120 * 1024 * 1024,
            flags={"XLA_TPU_FORCE_LP_LLO_SCHEDULER": True}),
    )(jnp.transpose(A_x.reshape(S, D)), A_wqkv, A_wo, B_w_gate, B_w_up, jnp.transpose(B_w_down))
    return jnp.transpose(out_t).reshape(1, S, D)
```
